```python
import jax
import jax.numpy as jnp

def _softmax(x, axis=-1):
    return jax.nn.softmax(x, axis=axis)
def _gelu(x):
    return jax.nn.gelu(x, approximate=True)
def _silu(x):
    return jax.nn.silu(x)
def _sigmoid(x):
    return jax.nn.sigmoid(x)
def _layernorm(x, axis=-1, eps=1e-5):
    m = jnp.mean(x, axis=axis, keepdims=True)
    v = jnp.var(x, axis=axis, keepdims=True)
    return (x - m) / jnp.sqrt(v + eps)
def _scatter_add(tgt, idx, src, axis=0):
    return tgt.at[idx].add(src)
def _segment_sum(src, seg, n):
    return jax.ops.segment_sum(src, seg, n)
class _Rng:
    def __init__(self, key):
        self._k = key
    def _next(self):
        self._k, sub = jax.random.split(self._k)
        return sub
    def normal(self, shape):
        return jax.random.normal(self._next(), shape, dtype=jnp.bfloat16)
    def randint(self, lo, hi, shape):
        return jax.random.randint(self._next(), shape, lo, hi, dtype=jnp.int32)
    def uniform(self, shape, lo=0.0, hi=1.0):
        return jax.random.uniform(self._next(), shape, jnp.bfloat16, lo, hi)
    def permutation(self, n):
        return jax.random.permutation(self._next(), n)


kernel_name = 'recurrent_scan__sliding_block_cached__glu_gated_glu__decode'

def setup_inputs():
    _rng = _Rng(jax.random.key(int.from_bytes(__import__("os").urandom(4), "little")))
    _w = (lambda a: (lambda t: t.astype(jnp.bfloat16) if jnp.issubdtype(t.dtype, jnp.floating) else t)(jnp.asarray(a)))
    def _A_setup():
        B, Sq, D = 1, 1, 576
        Hq, Hkv, Sk, Dh = 32, 16, 65536, 128
        assert Hq % Hkv == 0, (Hq, Hkv)
        return {
            "x": _w((lambda *s: _rng.normal(s) * 0.05)(B, Sq, D)),
            "k_cache": _w((lambda *s: _rng.normal(s) * 0.05)(B, Hkv, Sk, Dh)),
            "v_cache": _w((lambda *s: _rng.normal(s) * 0.05)(B, Hkv, Sk, Dh)),
            "wq": _w((lambda *s: _rng.normal(s) * 0.05)(D, Hq * Dh) * (D ** -0.5)),
            "wo": _w((lambda *s: _rng.normal(s) * 0.05)(Hq * Dh, D) * ((Hq * Dh) ** -0.5)),
        }
    _A_in = _A_setup()

    def _B_setup():
        B, S, D, F = 1, 1, 576, 4608
        return {
            "x": _w((lambda *s: _rng.normal(s) * 0.05)(B, S, D)),
            "w_gate": _w((lambda *s: _rng.normal(s) * 0.05)(D, F)),
            "w_up": _w((lambda *s: _rng.normal(s) * 0.05)(D, F)),
            "w_down": _w((lambda *s: _rng.normal(s) * 0.05)(F, D)),
        }
    _B_in = _B_setup()

    return {
        "A_x": _A_in["x"],
        "A_k_cache": _A_in["k_cache"],
        "A_v_cache": _A_in["v_cache"],
        "A_wq": _A_in["wq"],
        "A_wo": _A_in["wo"],
        "B_x": _B_in["x"],
        "B_w_gate": _B_in["w_gate"],
        "B_w_up": _B_in["w_up"],
        "B_w_down": _B_in["w_down"],
    }

def reference(A_x, A_k_cache, A_v_cache, A_wq, A_wo, B_x, B_w_gate, B_w_up, B_w_down):
    def _A_ref(x, k_cache, v_cache, wq, wo):
        B, Sq, D = x.shape
        Hq, Dh = 32, 128
        Hkv, Sk = k_cache.shape[1], k_cache.shape[2]
        W = min(4096, max(256, Sk // 4))
        rep = Hq // Hkv
        q = (lambda x, *d: x.transpose(*d))((x @ wq).reshape(B, Sq, Hq, Dh), 0, 2, 1, 3)
        k = jnp.repeat(k_cache[:, :, Sk - W:, :], rep, axis=1)
        v = jnp.repeat(v_cache[:, :, Sk - W:, :], rep, axis=1)
        scores = jnp.einsum("bhqd,bhkd->bhqk", q, k) * (Dh ** -0.5)
        p = _softmax(scores, axis=-1)
        o = jnp.einsum("bhqk,bhkd->bhqd", p, v)
        return (lambda x, *d: x.transpose(*d))(o, 0, 2, 1, 3).reshape(B, Sq, Hq * Dh) @ wo

    def _B_ref(x, w_gate, w_up, w_down):
        g = jnp.einsum("bsd,df->bsf", x, w_gate)
        u = jnp.einsum("bsd,df->bsf", x, w_up)
        h = _sigmoid(g) * u
        return jnp.einsum("bsf,fd->bsd", h, w_down)

    x = A_x
    xn = _layernorm(x, axis=-1)
    s = _A_ref(xn, A_k_cache, A_v_cache, A_wq, A_wo)
    g = _silu(_B_ref(xn, B_w_gate, B_w_up, B_w_down))
    return x + s * g
```

```python
import jax
import jax.numpy as jnp
import jax.experimental.pallas as pl
import jax.experimental.pallas.tpu as pltpu

HQ, DH = 32, 128
NT = (((1,), (1,)), ((), ()))
DEPTH = 3
FC = 512


def _kernel(x_h, k_h, v_h, wq_h, wo_h, wg_h, wu_h, wd_h, o_ref,
            xb, kb, vb, wqb, wob, wgb, wub, wdb, sems, xsem):
    HKV, W = kb.shape[0], kb.shape[1]
    SK = k_h.shape[2]
    D, F = wgb.shape
    NF = F // FC

    def attn_cps(j, slot):
        c = pl.ds(pl.multiple_of(j * 256, 256), 256)
        return [pltpu.make_async_copy(wq_h.at[:, c], wqb.at[:, c], sems.at[slot, 0]),
                pltpu.make_async_copy(k_h.at[0, j, pl.ds(SK - W, W), :], kb.at[j], sems.at[slot, 1]),
                pltpu.make_async_copy(v_h.at[0, j, pl.ds(SK - W, W), :], vb.at[j], sems.at[slot, 2]),
                pltpu.make_async_copy(wo_h.at[:, c], wob.at[:, c], sems.at[slot, 3])]

    def ffn_cps(i, slot):
        c = pl.ds(pl.multiple_of(i * FC, FC), FC)
        return [pltpu.make_async_copy(wg_h.at[:, c], wgb.at[:, c], sems.at[slot, 0]),
                pltpu.make_async_copy(wu_h.at[:, c], wub.at[:, c], sems.at[slot, 1]),
                pltpu.make_async_copy(wd_h.at[:, c], wdb.at[:, c], sems.at[slot, 2])]

    def start(cps):
        for n, c in enumerate(cps):
            c.start(priority=n % 2)

    xc = pltpu.make_async_copy(x_h, xb, xsem)
    xc.start()
    for s in range(DEPTH):
        start(attn_cps(s, s))
    xc.wait()
    x = xb[0].astype(jnp.float32)
    m = jnp.mean(x, axis=-1, keepdims=True)
    v = jnp.mean((x - m) ** 2, axis=-1, keepdims=True)
    xn = ((x - m) / jnp.sqrt(v + 1e-5)).astype(jnp.bfloat16)
    xn8 = jnp.broadcast_to(xn, (8, D))
    row = jax.lax.broadcasted_iota(jnp.int32, (8, DH), 0)

    def attn_body(j, acc):
        slot = j % DEPTH
        cps = attn_cps(j, slot)
        c = pl.ds(pl.multiple_of(j * 256, 256), 256)
        cps[0].wait()
        q = jnp.dot(xn8, wqb[:, c], preferred_element_type=jnp.float32)
        q = jnp.where(row == 0, q[:, :128], q[:, 128:]).astype(jnp.bfloat16)
        cps[1].wait()
        s = jax.lax.dot_general(q, kb[j], NT, preferred_element_type=jnp.float32) * (DH ** -0.5)
        mx = jnp.max(s, axis=-1, keepdims=True)
        p = jnp.exp(s - mx)
        l = jnp.sum(p, axis=-1, keepdims=True)
        cps[2].wait()
        o = jnp.dot(p.astype(jnp.bfloat16), vb[j], preferred_element_type=jnp.float32) / l
        o2 = jnp.concatenate([jnp.where(row == 0, o, 0.0), jnp.where(row == 1, o, 0.0)],
                             axis=1).astype(jnp.bfloat16)
        cps[3].wait()
        nxt = j + DEPTH

        @pl.when(nxt < HKV)
        def _():
            start(attn_cps(nxt, slot))

        @pl.when(nxt >= HKV)
        def _():
            start(ffn_cps(nxt - HKV, slot))

        return acc + jax.lax.dot_general(o2, wob[:, c], NT, preferred_element_type=jnp.float32)

    sacc = jax.lax.fori_loop(0, HKV, attn_body, jnp.zeros((8, D), jnp.float32))
    s_out = jnp.sum(sacc, axis=0, keepdims=True)

    def ffn_body(i, acc):
        slot = (i + HKV) % DEPTH
        cps = ffn_cps(i, slot)
        c = pl.ds(pl.multiple_of(i * FC, FC), FC)
        cps[0].wait()
        g = jnp.dot(xn8, wgb[:, c], preferred_element_type=jnp.float32)
        cps[1].wait()
        u = jnp.dot(xn8, wub[:, c], preferred_element_type=jnp.float32)
        h = (jax.nn.sigmoid(g) * u).astype(jnp.bfloat16)
        cps[2].wait()
        nxt = i + DEPTH

        @pl.when(nxt < NF)
        def _():
            start(ffn_cps(nxt, slot))

        return acc + jax.lax.dot_general(h, wdb[:, c], NT, preferred_element_type=jnp.float32)

    gacc = jax.lax.fori_loop(0, NF, ffn_body, jnp.zeros((8, D), jnp.float32))
    gg = gacc[0:1]
    gg = gg * jax.nn.sigmoid(gg)
    o_ref[0] = (x + s_out * gg).astype(o_ref.dtype)


@jax.jit
def pallas_recurrent_scan__sliding_block_cached__glu_gated_glu__decode_kernel(
    A_x, A_k_cache, A_v_cache, A_wq, A_wo, B_x, B_w_gate, B_w_up, B_w_down,
):
    del B_x
    D = A_x.shape[-1]
    HKV, SK = A_k_cache.shape[1], A_k_cache.shape[2]
    W = min(4096, max(256, SK // 4))
    F = B_w_gate.shape[1]
    bf = jnp.bfloat16
    return pl.pallas_call(
        _kernel,
        in_specs=[pl.BlockSpec(memory_space=pl.ANY)] * 8,
        out_specs=pl.BlockSpec(memory_space=pltpu.VMEM),
        out_shape=jax.ShapeDtypeStruct(A_x.shape, A_x.dtype),
        scratch_shapes=[
            pltpu.VMEM((1, 1, D), bf),
            pltpu.VMEM((HKV, W, DH), bf), pltpu.VMEM((HKV, W, DH), bf),
            pltpu.VMEM((D, HQ * DH), bf), pltpu.VMEM((D, HQ * DH), bf),
            pltpu.VMEM((D, F), bf), pltpu.VMEM((D, F), bf), pltpu.VMEM((D, F), bf),
            pltpu.SemaphoreType.DMA((DEPTH, 4)), pltpu.SemaphoreType.DMA(()),
        ],
        compiler_params=pltpu.CompilerParams(vmem_limit_bytes=100 * 1024 * 1024),
    )(A_x, A_k_cache, A_v_cache, A_wq, A_wo.T, B_w_gate, B_w_up, B_w_down.T)
```

```python
import jax
import jax.numpy as jnp
import jax.experimental.pallas as pl
import jax.experimental.pallas.tpu as pltpu

HQ, DH = 32, 128
NT = (((1,), (1,)), ((), ()))
DEPTH = 2
NSEM = 3 * DEPTH
FC = 512
OC = 512
LAST = (256, 256)
UNROLL = 8


def _kernel(x_h, k_h, v_h, wq_h, wo_h, wg_h, wu_h, wd_h, o_ref,
            xb, kb, vb, wqb, wob, wgb, wub, wdb, ob, sems):
    HKV, W = kb.shape[0], kb.shape[1]
    SK = k_h.shape[2]
    D, F = wgb.shape
    QC = 2 * DH
    NF = F // FC
    NOL = (HQ * DH - sum(LAST)) // OC
    assert HQ == 2 * HKV and F % FC == 0 and NOL * OC + sum(LAST) == HQ * DH
    assert NF >= DEPTH and NOL >= NSEM and len(LAST) <= NSEM and DEPTH % 2 == 0

    def issue(n, piece):
        u = UNROLL
        while n % u:
            u -= 2

        def body(i, c):
            for t in range(u):
                piece(i * u + t).start(priority=t % 2)
            return c

        jax.lax.fori_loop(0, n // u, body, 0)

    def w_start(h, b, c0, nc, r, sem):
        assert D % (2 * r) == 0
        c = pl.ds(c0, nc)

        def piece(i):
            rr = pl.ds(pl.multiple_of(i * r, r), r)
            return pltpu.make_async_copy(h.at[rr, c], b.at[rr, c], sem)

        issue(D // r, piece)

    def kv_start(h, b, j, sem):
        r = 128
        assert W % (2 * r) == 0

        def piece(i):
            o = pl.multiple_of(i * r, r)
            return pltpu.make_async_copy(
                h.at[0, j, pl.ds(SK - W + o, r), :], b.at[j, pl.ds(o, r), :], sem)

        issue(W // r, piece)

    def wait(dst, sem):
        pltpu.make_async_copy(dst, dst, sem).wait()

    def f0(i):
        return pl.multiple_of(i * FC, FC)

    def q0(j):
        return pl.multiple_of(j * QC, QC)

    def ffn_start(i, slot):
        w_start(wg_h, wgb, f0(i), FC, 16, sems.at[slot * 3])
        w_start(wu_h, wub, f0(i), FC, 16, sems.at[slot * 3 + 1])
        w_start(wd_h, wdb, f0(i), FC, 16, sems.at[slot * 3 + 2])

    def att_start(j, slot):
        w_start(wq_h, wqb, q0(j), QC, 48, sems.at[slot * 3])
        kv_start(k_h, kb, j, sems.at[slot * 3 + 1])
        kv_start(v_h, vb, j, sems.at[slot * 3 + 2])

    def wo_sem(i):
        return sems.at[((HKV + NF + i // 3) % DEPTH) * 3 + i % 3]

    def wo_start(i):
        w_start(wo_h, wob, pl.multiple_of(i * OC, OC), OC, 16, wo_sem(i))

    def wo_last_start(e):
        w_start(wo_h, wob, NOL * OC + sum(LAST[:e]), LAST[e], 48, wo_sem(NOL + e))

    xc = pltpu.make_async_copy(x_h, xb, sems.at[NSEM])
    xc.start()

    def prologue(s, c):
        ffn_start(s, s)
        return c

    jax.lax.fori_loop(0, DEPTH, prologue, 0)

    xc.wait()
    x = xb[0].astype(jnp.float32)
    m = jnp.mean(x, axis=-1, keepdims=True)
    v = jnp.mean((x - m) ** 2, axis=-1, keepdims=True)
    xn = ((x - m) / jnp.sqrt(v + 1e-5)).astype(jnp.bfloat16)
    xn8 = jnp.broadcast_to(xn, (8, D))
    row = jax.lax.broadcasted_iota(jnp.int32, (8, DH), 0)

    def ffn_body(i, acc):
        slot = i % DEPTH
        c = pl.ds(f0(i), FC)
        wait(wgb.at[:, c], sems.at[slot * 3])
        g = jnp.dot(xn8, wgb[:, c], preferred_element_type=jnp.float32)
        wait(wub.at[:, c], sems.at[slot * 3 + 1])
        u = jnp.dot(xn8, wub[:, c], preferred_element_type=jnp.float32)
        h = (jax.nn.sigmoid(g) * u).astype(jnp.bfloat16)
        wait(wdb.at[:, c], sems.at[slot * 3 + 2])
        nxt = i + DEPTH

        @pl.when(nxt < NF)
        def _():
            ffn_start(nxt, slot)

        @pl.when(nxt >= NF)
        def _():
            att_start(nxt - NF, slot)

        return acc + jax.lax.dot_general(h, wdb[:, c], NT, preferred_element_type=jnp.float32)

    gacc = jax.lax.fori_loop(0, NF, ffn_body, jnp.zeros((8, D), jnp.float32))
    gate = gacc * jax.nn.sigmoid(gacc)

    def attn_body(j, carry):
        slot = (j + NF) % DEPTH
        c = pl.ds(q0(j), QC)
        wait(wqb.at[:, c], sems.at[slot * 3])
        q = jnp.dot(xn8, wqb[:, c], preferred_element_type=jnp.float32)
        q = jnp.where(row == 0, q[:, :DH], q[:, DH:]).astype(jnp.bfloat16)
        wait(kb.at[j], sems.at[slot * 3 + 1])
        s = jax.lax.dot_general(q, kb[j], NT, preferred_element_type=jnp.float32) * (DH ** -0.5)
        mx = jnp.max(s, axis=-1, keepdims=True)
        p = jnp.exp(s - mx)
        l = jnp.sum(p, axis=-1, keepdims=True)
        wait(vb.at[j], sems.at[slot * 3 + 2])
        nxt = j + DEPTH

        @pl.when(nxt < HKV)
        def _():
            att_start(nxt, slot)

        @pl.when(nxt >= HKV)
        def _():
            def b(t, cc):
                wo_start((nxt - HKV) * 3 + t)
                return cc

            jax.lax.fori_loop(0, 3, b, 0)

        o = jnp.dot(p.astype(jnp.bfloat16), vb[j], preferred_element_type=jnp.float32) / l
        ob[:, c] = jnp.concatenate(
            [jnp.broadcast_to(o[0:1], (8, DH)), jnp.broadcast_to(o[1:2], (8, DH))], axis=1)
        return carry

    jax.lax.fori_loop(0, HKV, attn_body, 0)

    def wo_body(i, acc):
        c = pl.ds(pl.multiple_of(i * OC, OC), OC)
        oc = ob[:, c].astype(jnp.bfloat16)
        wait(wob.at[:, c], wo_sem(i))
        nxt = i + NSEM

        @pl.when(nxt < NOL)
        def _():
            wo_start(nxt)

        for e in range(len(LAST)):
            @pl.when(nxt == NOL + e)
            def _():
                wo_last_start(e)

        return acc + jax.lax.dot_general(oc, wob[:, c], NT, preferred_element_type=jnp.float32)

    sacc = jax.lax.fori_loop(0, NOL, wo_body, jnp.zeros((8, D), jnp.float32))
    for e in range(len(LAST)):
        c = pl.ds(NOL * OC + sum(LAST[:e]), LAST[e])
        oc = ob[:, c].astype(jnp.bfloat16)
        wait(wob.at[:, c], wo_sem(NOL + e))
        sacc = sacc + jax.lax.dot_general(oc, wob[:, c], NT, preferred_element_type=jnp.float32)

    o_ref[0] = (x + sacc[0:1] * gate[0:1]).astype(o_ref.dtype)


@jax.jit
def pallas_recurrent_scan__sliding_block_cached__glu_gated_glu__decode_kernel(
    A_x, A_k_cache, A_v_cache, A_wq, A_wo, B_x, B_w_gate, B_w_up, B_w_down,
):
    del B_x
    D = A_x.shape[-1]
    HKV, SK = A_k_cache.shape[1], A_k_cache.shape[2]
    W = min(4096, max(256, SK // 4))
    F = B_w_gate.shape[1]
    bf = jnp.bfloat16
    return pl.pallas_call(
        _kernel,
        in_specs=[pl.BlockSpec(memory_space=pl.ANY)] * 8,
        out_specs=pl.BlockSpec(memory_space=pltpu.VMEM),
        out_shape=jax.ShapeDtypeStruct(A_x.shape, A_x.dtype),
        scratch_shapes=[
            pltpu.VMEM((1, 1, D), bf),
            pltpu.VMEM((HKV, W, DH), bf), pltpu.VMEM((HKV, W, DH), bf),
            pltpu.VMEM((D, HQ * DH), bf), pltpu.VMEM((D, HQ * DH), bf),
            pltpu.VMEM((D, F), bf), pltpu.VMEM((D, F), bf), pltpu.VMEM((D, F), bf),
            pltpu.VMEM((8, HQ * DH), jnp.float32),
            pltpu.SemaphoreType.DMA((NSEM + 1,)),
        ],
        compiler_params=pltpu.CompilerParams(vmem_limit_bytes=100 * 1024 * 1024),
    )(A_x, A_k_cache, A_v_cache, A_wq, A_wo.T, B_w_gate, B_w_up, B_w_down.T)
```
